```python
import os as _os
_os.environ.setdefault("JAX_PLATFORMS", "cpu")
import jax
import jax.numpy as jnp

def _softmax(x, axis=-1):
    return jax.nn.softmax(x, axis=axis)
def _gelu(x):
    return jax.nn.gelu(x, approximate=True)
def _silu(x):
    return jax.nn.silu(x)
def _sigmoid(x):
    return jax.nn.sigmoid(x)
def _layernorm(x, axis=-1, eps=1e-5):
    m = jnp.mean(x, axis=axis, keepdims=True)
    v = jnp.var(x, axis=axis, keepdims=True)
    return (x - m) / jnp.sqrt(v + eps)
def _scatter_add(tgt, idx, src, axis=0):
    return tgt.at[idx].add(src)
def _segment_sum(src, seg, n):
    return jax.ops.segment_sum(src, seg, n)
class _Rng:
    def __init__(self, key):
        self._k = key
    def _next(self):
        self._k, sub = jax.random.split(self._k)
        return sub
    def normal(self, shape):
        return jax.random.normal(self._next(), shape, dtype=jnp.bfloat16)
    def randint(self, lo, hi, shape):
        return jax.random.randint(self._next(), shape, lo, hi, dtype=jnp.int32)
    def uniform(self, shape, lo=0.0, hi=1.0):
        return jax.random.uniform(self._next(), shape, jnp.bfloat16, lo, hi)
    def permutation(self, n):
        return jax.random.permutation(self._next(), n)


kernel_name = 'gated_mix__ssm_conv_h3__ssm_conv_h3__prompt'

def setup_inputs():
    _rng = _Rng(jax.random.key(int.from_bytes(__import__("os").urandom(4), "little")))
    _w = (lambda a: (lambda t: t.astype(jnp.bfloat16) if jnp.issubdtype(t.dtype, jnp.floating) else t)(jnp.asarray(a)))
    def _A_setup():
        B, S, D = 1, 2048, 640
        ks = 4
        return {
            "q": _w((lambda *s: _rng.normal(s) * 0.05)(B, S, D)),
            "k": _w((lambda *s: _rng.normal(s) * 0.05)(B, S, D)),
            "v": _w((lambda *s: _rng.normal(s) * 0.05)(B, S, D)),
            "shift_k": _w((lambda *s: _rng.normal(s) * 0.05)(D, ks) * 0.5),
            "ssm_k": _w((lambda *s: _rng.normal(s) * 0.05)(D, S) * (1.0 / S ** 0.5)),
            "ssm_D": _w((lambda *s: _rng.normal(s) * 0.05)(D)),
        }
    _A_in = _A_setup()

    def _B_setup():
        B, S, D = 1, 2048, 640
        ks = 4
        return {
            "q": _w((lambda *s: _rng.normal(s) * 0.05)(B, S, D)),
            "k": _w((lambda *s: _rng.normal(s) * 0.05)(B, S, D)),
            "v": _w((lambda *s: _rng.normal(s) * 0.05)(B, S, D)),
            "shift_k": _w((lambda *s: _rng.normal(s) * 0.05)(D, ks) * 0.5),
            "ssm_k": _w((lambda *s: _rng.normal(s) * 0.05)(D, S) * (1.0 / S ** 0.5)),
            "ssm_D": _w((lambda *s: _rng.normal(s) * 0.05)(D)),
        }
    _B_in = _B_setup()

    return {
        "A_q": _A_in["q"],
        "A_k": _A_in["k"],
        "A_v": _A_in["v"],
        "A_shift_k": _A_in["shift_k"],
        "A_ssm_k": _A_in["ssm_k"],
        "A_ssm_D": _A_in["ssm_D"],
        "B_q": _B_in["q"],
        "B_k": _B_in["k"],
        "B_v": _B_in["v"],
        "B_shift_k": _B_in["shift_k"],
        "B_ssm_k": _B_in["ssm_k"],
        "B_ssm_D": _B_in["ssm_D"],
        "gate_w": _w((lambda *s: _rng.normal(s) * 0.05)(640) * 16.0),
    }

def reference(A_q, A_k, A_v, A_shift_k, A_ssm_k, A_ssm_D, B_q, B_k, B_v, B_shift_k, B_ssm_k, B_ssm_D, gate_w):
    def _A_ref(q, k, v, shift_k, ssm_k, ssm_D):
        B, S, D = q.shape
        ks = shift_k.shape[-1]
        k_pad = jnp.pad(k, ((0, 0), (ks - 1, 0), (0, 0)))
        k_shift = jnp.zeros_like(k)
        for t in range(ks):
            k_shift = k_shift + k_pad[:, t:t + S, :] * shift_k[:, ks - 1 - t][None, None, :]
        kv = k_shift * v
        L = 2 * S
        kv_pad = jnp.pad(kv, ((0, 0), (0, S), (0, 0)))
        kf_pad = jnp.pad(ssm_k, ((0, 0), (0, S)))
        kv_f = (lambda x, axes=(-2,-1): jnp.fft.rfft2(x.astype(jnp.float32), axes=axes))(kv_pad[:, None, :, :], axes=(1, 2))
        kf_f = (lambda x, axes=(-2,-1): jnp.fft.rfft2(x.astype(jnp.float32), axes=axes))(kf_pad[:, None, :], axes=(1, 2))
        kf_f = (lambda x, *d: x.transpose(*d))(kf_f, 1, 2, 0)
        y_f = kv_f * kf_f[None, :, :, :]
        y = (lambda x, s, axes=(-2,-1): jnp.fft.irfft2(x, s=s, axes=axes).astype(jnp.bfloat16))(y_f, (1, L), axes=(1, 2))[:, 0, :S, :]
        y = y + kv * ssm_D[None, None, :]
        return q * y

    def _B_ref(q, k, v, shift_k, ssm_k, ssm_D):
        B, S, D = q.shape
        ks = shift_k.shape[-1]
        k_pad = jnp.pad(k, ((0, 0), (ks - 1, 0), (0, 0)))
        k_shift = jnp.zeros_like(k)
        for t in range(ks):
            k_shift = k_shift + k_pad[:, t:t + S, :] * shift_k[:, ks - 1 - t][None, None, :]
        kv = k_shift * v
        L = 2 * S
        kv_pad = jnp.pad(kv, ((0, 0), (0, S), (0, 0)))
        kf_pad = jnp.pad(ssm_k, ((0, 0), (0, S)))
        kv_f = (lambda x, axes=(-2,-1): jnp.fft.rfft2(x.astype(jnp.float32), axes=axes))(kv_pad[:, None, :, :], axes=(1, 2))
        kf_f = (lambda x, axes=(-2,-1): jnp.fft.rfft2(x.astype(jnp.float32), axes=axes))(kf_pad[:, None, :], axes=(1, 2))
        kf_f = (lambda x, *d: x.transpose(*d))(kf_f, 1, 2, 0)
        y_f = kv_f * kf_f[None, :, :, :]
        y = (lambda x, s, axes=(-2,-1): jnp.fft.irfft2(x, s=s, axes=axes).astype(jnp.bfloat16))(y_f, (1, L), axes=(1, 2))[:, 0, :S, :]
        y = y + kv * ssm_D[None, None, :]
        return q * y

    x = A_q
    g = _sigmoid((x * gate_w).sum(-1, keepdims=True))
    a = _A_ref(x, A_k, A_v, A_shift_k, A_ssm_k, A_ssm_D)
    b = _B_ref(x, B_k, B_v, B_shift_k, B_ssm_k, B_ssm_D)
    return g * a + (1 - g) * b
```

```python
import jax
import jax.numpy as jnp
from jax import lax
import jax.experimental.pallas as pl
import jax.experimental.pallas.tpu as pltpu

S = 2048
DB = 128
NB = 5
UNROLL = 4
GPB = 10
CH = 256
NOFF = 8
F32 = jnp.float32
BF16 = jnp.bfloat16
U32 = jnp.uint32


def _rb(x):
    return x.astype(BF16).astype(F32)


def _kernel(q_hbm, ka_hbm, va_hbm, kb_hbm, vb_hbm, ha_hbm, hb_hbm,
            gw_ref, sk_ref, dd_ref,
            o_hbm,
            q_s, kv_in, h_in, o_s, g_s, kpad_s, kvw_s,
            xt0_s, xt1_s, hw0_s, hw1_s, yt_s, yw_s,
            a0_s, a1_s, b0_s, b1_s, c0_s, c1_s, sh_s,
            sem_q, sem_kv, sem_h, sem_o):
    a_bufs = (a0_s, a1_s)
    b_bufs = (b0_s, b1_s)
    c_bufs = (c0_s, c1_s)
    xt_bufs = (xt0_s, xt1_s)
    hw_bufs = (hw0_s, hw1_s)
    nch = S // CH

    def kv_copy(a, p):
        src = (ka_hbm, va_hbm, kb_hbm, vb_hbm)[a]
        return pltpu.make_async_copy(src.at[:, pl.ds(p * DB, DB)], kv_in.at[a, p], sem_kv.at[a, p])

    def h_copy(br, p):
        src = (ha_hbm, hb_hbm)[br]
        return pltpu.make_async_copy(src.at[pl.ds(p * DB, DB), :], h_in.at[br, p], sem_h.at[br, p])

    def q_copy():
        return pltpu.make_async_copy(q_hbm, q_s, sem_q.at[0])

    def o_copy(p):
        return pltpu.make_async_copy(o_s.at[p], o_hbm.at[:, pl.ds(p * DB, DB)], sem_o.at[p])

    for p in range(NB):
        for br in range(2):
            kv_copy(2 * br, p).start()
            kv_copy(2 * br + 1, p).start()
            h_copy(br, p).start()
        if p == 1:
            q_copy().start()

    lane = lax.broadcasted_iota(jnp.int32, (8, 128), 1)
    sub = lax.broadcasted_iota(jnp.int32, (8, 128), 0)
    lane16 = lax.broadcasted_iota(jnp.int32, (16, 128), 1)
    lane_hd = lax.broadcasted_iota(jnp.int32, (DB // 2, 128), 1)
    tri = lane < 2 * sub
    rr = lax.broadcasted_iota(jnp.int32, (128, 128), 0)
    cc = lax.broadcasted_iota(jnp.int32, (128, 128), 1)
    for i in range(NOFF):
        sh_s[i] = jnp.where(cc == rr + (16 - NOFF + i), 1.0, 0.0).astype(BF16)

    def gate():
        w = gw_ref[...].astype(F32)
        ones = jnp.ones((gw_ref.shape[1], DB), BF16)

        def body(c, carry):
            r0 = pl.multiple_of(c * CH, CH)
            x = q_s[pl.ds(r0, CH), :].astype(F32)
            pr = (x * w).astype(BF16)
            s = _rb(jnp.dot(pr, ones, preferred_element_type=F32))
            g_s[pl.ds(r0, CH), :] = _rb(jax.nn.sigmoid(s))
            return carry
        lax.fori_loop(0, nch, body, 0)

    def kv_cp(p, br):
        kpad_s[br, pl.ds(0, 8), :] = jnp.zeros((8, DB), F32)

        def cp(c, carry):
            r0 = pl.multiple_of(c * CH, CH)
            kpad_s[br, pl.ds(r0 + 8, CH), :] = kv_in[2 * br, p, pl.ds(r0, CH), :].astype(F32)
            return carry
        lax.fori_loop(0, nch, cp, 0)

    def kv_chunk(p, br, c):
        w = sk_ref[br, :, pl.ds(p * DB, DB)].astype(F32)
        r0 = c * CH if isinstance(c, int) else pl.multiple_of(c * CH, CH)
        r1 = c * (CH // 2) if isinstance(c, int) else pl.multiple_of(c * (CH // 2), CH // 2)
        acc = kpad_s[br, pl.ds(r0 + 5, CH), :] * w[3:4]
        acc = acc + kpad_s[br, pl.ds(r0 + 6, CH), :] * w[2:3]
        acc = acc + kpad_s[br, pl.ds(r0 + 7, CH), :] * w[1:2]
        acc = acc + kpad_s[br, pl.ds(r0 + 8, CH), :] * w[0:1]
        v = kv_in[2 * br + 1, p, pl.ds(r0, CH), :].astype(F32)
        kv = (_rb(acc) * v).astype(BF16)
        wd = pltpu.bitcast(kv, U32)
        wd = (wd >> 16) | (wd << 16)
        kvw_s[br, pl.ds(r1, CH // 2), :] = wd

    def x_tr(p, br, m):
        blk = kvw_s[br, pl.ds(m, 128, stride=8), :]
        blk_t = pltpu.bitcast(pltpu.bitcast(blk, F32).T, U32)
        xt_bufs[p % 2][pl.ds((br * 8 + 7 - m) * 128, 128), :] = blk_t

    def h_slab(p, br, gq):
        hw_s = hw_bufs[p % 2]
        hp = pltpu.bitcast(h_in[br, p, :, pl.ds(gq * 128, 128)], U32)
        if gq == 0:
            prev = jnp.zeros((DB // 2, 128), U32)
        else:
            prev = pltpu.bitcast(h_in[br, p, :, pl.ds((gq - 1) * 128, 128)], U32)
        h1 = pltpu.roll(jnp.where(lane_hd == 127, prev, hp), 1, 1)
        base = (br * 16 + gq) * DB
        hw_s[pl.ds(base, DB // 2), :] = (h1 & jnp.uint32(0xFFFF)) | (hp << 16)
        hw_s[pl.ds(base + DB // 2, DB // 2), :] = (h1 >> 16) | (hp & jnp.uint32(0xFFFF0000))

    def prep(p):
        wait_inputs(p, 0)
        kv_cp(p, 0)

        def kv0(c, carry):
            kv_chunk(p, 0, c)
            return carry
        lax.fori_loop(0, nch, kv0, 0)
        wait_inputs(p, 1)
        kv_cp(p, 1)
        for c in range(nch):
            x_tr(p, 0, c)
            kv_chunk(p, 1, c)
            h_slab(p, 0, 2 * c)
            h_slab(p, 0, 2 * c + 1)
        for c in range(nch):
            x_tr(p, 1, c)
            h_slab(p, 1, 2 * c)
            h_slab(p, 1, 2 * c + 1)

    def wait_inputs(p, br):
        kv_copy(2 * br, p).wait()
        kv_copy(2 * br + 1, p).wait()
        h_copy(br, p).wait()

    def post(p):
        for br in range(2):
            for i in range(8):
                blk = yt_s[pl.ds((br * 8 + i) * 128, 128), :]
                blk_t = pltpu.bitcast(pltpu.bitcast(blk, F32).T, U32)
                yw_s[br, pl.ds(7 - i, 128, stride=8), :] = blk_t

        def ep(c, carry):
            r0 = pl.multiple_of(c * CH, CH)
            r1 = pl.multiple_of(c * (CH // 2), CH // 2)
            q = q_s[pl.ds(r0, CH), pl.ds(p * DB, DB)].astype(F32)
            g = g_s[pl.ds(r0, CH), :]
            ya = pltpu.bitcast(yw_s[0, pl.ds(r1, CH // 2), :], BF16).astype(F32)
            yb = pltpu.bitcast(yw_s[1, pl.ds(r1, CH // 2), :], BF16).astype(F32)
            res = q * (yb + g * (ya - yb))
            o_s[p, pl.ds(r0, CH), :] = res.astype(BF16)
            return carry
        lax.fori_loop(0, nch, ep, 0)

    def stage1(pblk, grp, slot):
        a_s, b_s = a_bufs[slot], b_bufs[slot]
        xt_s, hw_s = xt_bufs[pblk % 2], hw_bufs[pblk % 2]
        xws = []
        for u in range(UNROLL):
            c = grp * UNROLL + u
            br = c // DB
            d = c % DB
            hrow = (d % 2) * (DB // 2) + d // 2
            rprev = None
            for gq in range(16):
                cur = jnp.broadcast_to(hw_s[pl.ds((br * 16 + gq) * DB + hrow, 1), :], (8, 128))
                rc = pltpu.roll(cur, 0, 1, stride=2, stride_axis=0)
                a = jnp.where(tri, jnp.uint32(0) if rprev is None else rprev, rc)
                a_s[u, pl.ds(8 * (gq // 2), 8), pl.ds(128 * (gq % 2), 128)] = a
                rprev = rc
            xw = xt_s[pl.ds(br * 8 * DB + d, 8, stride=128), :]
            b_s[u, pl.ds(0, 8), :] = xw
            xws.append(xw)
            for p in range(1, 16 - NOFF):
                b_s[u, pl.ds(8 * p, 8), :] = jnp.where(lane < p, jnp.uint32(0), pltpu.roll(xw, p, 1))
        if NOFF:
            xall = pltpu.bitcast(jnp.concatenate(xws, axis=0), BF16)
            for i in range(NOFF):
                p = 16 - NOFF + i
                sh = jnp.dot(xall, sh_s[i], preferred_element_type=F32).astype(BF16)
                shw = pltpu.bitcast(sh, U32)
                for u in range(UNROLL):
                    b_s[u, pl.ds(8 * p, 8), :] = shw[8 * u:8 * u + 8]

    def stage2(slot):
        a_s, b_s, c_s = a_bufs[slot], b_bufs[slot], c_bufs[slot]
        for u in range(UNROLL):
            am = pltpu.bitcast(a_s[u], BF16)
            bm = pltpu.bitcast(b_s[u], BF16)
            c_s[u] = jnp.dot(am, bm, preferred_element_type=F32)

    def stage3(pblk, grp, slot):
        c_s = c_bufs[slot]
        xt_s = xt_bufs[pblk % 2]
        for u in range(UNROLL):
            c = grp * UNROLL + u
            br = c // DB
            d = c % DB
            parts = [c_s[u, pl.ds(0, 16), :]]
            for g in range(1, 8):
                o = c_s[u, pl.ds(16 * g, 16), :]
                parts.append(jnp.where(lane16 < 16 * g, 0.0, pltpu.roll(o, 16 * g, 1)))
            while len(parts) > 1:
                parts = [parts[i] + parts[i + 1] for i in range(0, len(parts), 2)]
            xw = xt_s[pl.ds(br * 8 * DB + d, 8, stride=128), :]
            xw = (xw >> 16) | (xw << 16)
            xf = pltpu.bitcast(xw, BF16).astype(F32)
            dv = jnp.broadcast_to(dd_ref[pl.ds(br * (NB * DB) + pblk * DB + d, 1), :], (16, 128))
            y = parts[0] + xf * dv
            yt_s[pl.ds(br * 8 * DB + d, 8, stride=128), :] = pltpu.bitcast(y.astype(BF16), U32)

    G = 2 * DB // UNROLL

    def chan_loop(p):
        def body(j, carry):
            for z in range(GPB):
                it = GPB * j + z + 2
                s0 = z % 2
                stage1(p, it, s0)
                stage2(1 - s0)
                stage3(p, it - 2, s0)
            return carry
        lax.fori_loop(0, (G - 2) // GPB, body, 0)
        for it in range(2 + ((G - 2) // GPB) * GPB, G + 2):
            s0 = it % 2
            if it < G:
                stage1(p, it, s0)
            elif p + 1 < NB:
                stage1(p + 1, it - G, s0)
            if it < G + 1 or p + 1 < NB:
                stage2(1 - s0)
            stage3(p, it - 2, s0)

    prep(0)
    stage1(0, 0, 0)
    stage1(0, 1, 1)
    stage2(0)
    for p in range(NB):
        if p + 1 < NB:
            prep(p + 1)
        chan_loop(p)
        if p == 0:
            q_copy().wait()
            gate()
        post(p)
        o_copy(p).start()
    for p in range(NB):
        o_copy(p).wait()


@jax.jit
def pallas_gated_mix__ssm_conv_h3__ssm_conv_h3__prompt_kernel(
    A_q, A_k, A_v, A_shift_k, A_ssm_k, A_ssm_D,
    B_q, B_k, B_v, B_shift_k, B_ssm_k, B_ssm_D, gate_w,
):
    B, S_, D = A_q.shape
    assert B == 1 and S_ == S and D == NB * DB
    sk = jnp.stack([A_shift_k.T, B_shift_k.T])
    dd = jnp.broadcast_to(jnp.concatenate([A_ssm_D, B_ssm_D]).astype(F32)[:, None], (2 * D, 128))
    args = [A_q.reshape(S, D), A_k.reshape(S, D), A_v.reshape(S, D),
            B_k.reshape(S, D), B_v.reshape(S, D), A_ssm_k, B_ssm_k,
            gate_w.reshape(1, D), sk, dd]
    any_spec = pl.BlockSpec(memory_space=pl.ANY)
    vmem_spec = pl.BlockSpec(memory_space=pltpu.VMEM)
    in_specs = [any_spec] * 7 + [vmem_spec] * 3
    scratch = [
        pltpu.VMEM((S, D), BF16),
        pltpu.VMEM((4, NB, S, DB), BF16),
        pltpu.VMEM((2, NB, DB, S), BF16),
        pltpu.VMEM((NB, S, DB), BF16),
        pltpu.VMEM((S, DB), F32),
        pltpu.VMEM((2, S + 8, DB), F32),
        pltpu.VMEM((2, S // 2, DB), U32),
        pltpu.VMEM((2 * 8 * DB, 128), U32),
        pltpu.VMEM((2 * 8 * DB, 128), U32),
        pltpu.VMEM((2 * 16 * DB, 128), U32),
        pltpu.VMEM((2 * 16 * DB, 128), U32),
        pltpu.VMEM((2 * 8 * DB, 128), U32),
        pltpu.VMEM((2, S // 2, DB), U32),
        pltpu.VMEM((UNROLL, 64, 256), U32),
        pltpu.VMEM((UNROLL, 64, 256), U32),
        pltpu.VMEM((UNROLL, 128, 128), U32),
        pltpu.VMEM((UNROLL, 128, 128), U32),
        pltpu.VMEM((UNROLL, 128, 128), F32),
        pltpu.VMEM((UNROLL, 128, 128), F32),
        pltpu.VMEM((max(NOFF, 1), 128, 128), BF16),
        pltpu.SemaphoreType.DMA((1,)),
        pltpu.SemaphoreType.DMA((4, NB)),
        pltpu.SemaphoreType.DMA((2, NB)),
        pltpu.SemaphoreType.DMA((NB,)),
    ]
    out = pl.pallas_call(
        _kernel,
        in_specs=in_specs,
        out_specs=pl.BlockSpec(memory_space=pl.ANY),
        out_shape=jax.ShapeDtypeStruct((S, D), BF16),
        scratch_shapes=scratch,
        compiler_params=pltpu.CompilerParams(vmem_limit_bytes=100 * 1024 * 1024),
    )(*args)
    return out.reshape(1, S, D)
```
